```python
import jax
import jax.numpy as jnp

def _softmax(x, axis=-1):
    return jax.nn.softmax(x, axis=axis)

def _gelu(x):
    return jax.nn.gelu(x, approximate=True)

def _silu(x):
    return jax.nn.silu(x)

def _sigmoid(x):
    return jax.nn.sigmoid(x)

def _layernorm(x, axis=-1, eps=1e-05):
    m = jnp.mean(x, axis=axis, keepdims=True)
    v = jnp.var(x, axis=axis, keepdims=True)
    return (x - m) / jnp.sqrt(v + eps)

def _scatter_add(tgt, idx, src, axis=0):
    return tgt.at[idx].add(src)

def _segment_sum(src, seg, n):
    return jax.ops.segment_sum(src, seg, n)

class _Rng:

    def __init__(self, key):
        self._k = key

    def _next(self):
        self._k, sub = jax.random.split(self._k)
        return sub

    def normal(self, shape):
        return jax.random.normal(self._next(), shape, dtype=jnp.bfloat16)

    def randint(self, lo, hi, shape):
        return jax.random.randint(self._next(), shape, lo, hi, dtype=jnp.int32)

    def uniform(self, shape, lo=0.0, hi=1.0):
        return jax.random.uniform(self._next(), shape, jnp.bfloat16, lo, hi)

    def permutation(self, n):
        return jax.random.permutation(self._next(), n)
kernel_name = 'adaLN_cond__sliding_block_cached__geglu_ffn__decode'

def setup_inputs():
    _rng = _Rng(jax.random.key(int.from_bytes(__import__("os").urandom(4), "little")))
    _w = lambda a: (lambda t: t.astype(jnp.bfloat16) if jnp.issubdtype(t.dtype, jnp.floating) else t)(jnp.asarray(a))

    def _A_setup():
        B, Sq, D = (1, 1, 640)
        Hq, Hkv, Sk, Dh = (32, 32, 32768, 192)
        assert Hq % Hkv == 0, (Hq, Hkv)
        return {'x': _w((lambda *s: _rng.normal(s) * 0.05)(B, Sq, D)), 'k_cache': _w((lambda *s: _rng.normal(s) * 0.05)(B, Hkv, Sk, Dh)), 'v_cache': _w((lambda *s: _rng.normal(s) * 0.05)(B, Hkv, Sk, Dh)), 'wq': _w((lambda *s: _rng.normal(s) * 0.05)(D, Hq * Dh) * D ** (-0.5)), 'wo': _w((lambda *s: _rng.normal(s) * 0.05)(Hq * Dh, D) * (Hq * Dh) ** (-0.5))}
    _A_in = _A_setup()

    def _B_setup():
        B, S, D, F = (1, 1, 640, 1536)
        return {'x': _w((lambda *s: _rng.normal(s) * 0.05)(B, S, D)), 'w_gate': _w((lambda *s: _rng.normal(s) * 0.05)(D, F)), 'w_up': _w((lambda *s: _rng.normal(s) * 0.05)(D, F)), 'w_down': _w((lambda *s: _rng.normal(s) * 0.05)(F, D))}
    _B_in = _B_setup()
    return {'A_x': _A_in['x'], 'A_k_cache': _A_in['k_cache'], 'A_v_cache': _A_in['v_cache'], 'A_wq': _A_in['wq'], 'A_wo': _A_in['wo'], 'B_x': _B_in['x'], 'B_w_gate': _B_in['w_gate'], 'B_w_up': _B_in['w_up'], 'B_w_down': _B_in['w_down'], 'c': _w((lambda *s: _rng.normal(s) * 0.05)(1, 640)), 'w_mod': _w((lambda *s: _rng.normal(s) * 0.05)(640, 6 * 640) * 640 ** (-0.5))}

def reference(A_x, A_k_cache, A_v_cache, A_wq, A_wo, B_x, B_w_gate, B_w_up, B_w_down, c, w_mod):

    def _A_ref(x, k_cache, v_cache, wq, wo):
        B, Sq, D = x.shape
        Hq, Dh = (32, 192)
        Hkv, Sk = (k_cache.shape[1], k_cache.shape[2])
        W = min(4096, max(256, Sk // 4))
        rep = Hq // Hkv
        q = (lambda x, *d: x.transpose(*d))((x @ wq).reshape(B, Sq, Hq, Dh), 0, 2, 1, 3)
        k = jnp.repeat(k_cache[:, :, Sk - W:, :], rep, axis=1)
        v = jnp.repeat(v_cache[:, :, Sk - W:, :], rep, axis=1)
        scores = jnp.einsum('bhqd,bhkd->bhqk', q, k) * Dh ** (-0.5)
        p = _softmax(scores, axis=-1)
        o = jnp.einsum('bhqk,bhkd->bhqd', p, v)
        return (lambda x, *d: x.transpose(*d))(o, 0, 2, 1, 3).reshape(B, Sq, Hq * Dh) @ wo

    def _B_ref(x, w_gate, w_up, w_down):
        return _gelu(x @ w_gate) * (x @ w_up) @ w_down
    x = A_x
    mod = (_silu(c) @ w_mod).reshape(c.shape[0], 6, 1, -1)
    sa, ca, ga, sb, cb, gb = (mod[:, 0].copy(), mod[:, 1].copy(), mod[:, 2].copy(), mod[:, 3].copy(), mod[:, 4].copy(), mod[:, 5].copy())
    h = _layernorm(x, axis=-1) * (1 + ca) + sa
    x = x + ga * _A_ref(h, A_k_cache, A_v_cache, A_wq, A_wo)
    h = _layernorm(x, axis=-1) * (1 + cb) + sb
    x = x + gb * _B_ref(h, B_w_gate, B_w_up, B_w_down)
    return x
```

```python
import functools
import jax
import jax.numpy as jnp
from jax import lax
import jax.experimental.pallas as pl
import jax.experimental.pallas.tpu as pltpu

D = 640
H = 32
DH = 192
SK = 32768
W = min(4096, max(256, SK // 4))
F = 1536
NP = H // 2
NB = 4
EPS = 1e-5
f32 = jnp.float32
bf16 = jnp.bfloat16


def _ln(x):
    m = jnp.mean(x, axis=-1, keepdims=True)
    d = x - m
    v = jnp.mean(d * d, axis=-1, keepdims=True)
    return d / jnp.sqrt(v + EPS)


def _rows(x):
    return jnp.broadcast_to(x, (8, x.shape[-1]))


def _dot(a, b):
    return jnp.dot(a, b, preferred_element_type=f32)


def _r(x):
    return x.astype(bf16).astype(f32)


def _kernel(mode, x_hbm, c_hbm, k_hbm, v_hbm, wq_hbm, wo_hbm, wm_hbm, wg_hbm, wu_hbm, wd_hbm,
            o_ref,
            x_v, c_v, wm_v, wq_v, k_v, v_v, wo_v, wg_v, wu_v, wd_v,
            s_misc, s_wq, s_k, s_v, s_wo):
    HM = 3 * D

    def pair_copies(j, slot):
        h0 = 2 * j
        return (
            pltpu.make_async_copy(wq_hbm.at[:, pl.ds(pl.multiple_of(j * 2 * DH, 128), 2 * DH)], wq_v.at[slot], s_wq.at[slot]),
            pltpu.make_async_copy(k_hbm.at[pl.ds(h0, 2), :, pl.ds(SK - W, W)], k_v.at[slot], s_k.at[slot]),
            pltpu.make_async_copy(v_hbm.at[pl.ds(h0, 2), :, pl.ds(SK - W, W)], v_v.at[slot], s_v.at[slot]),
            pltpu.make_async_copy(wo_hbm.at[pl.ds(pl.multiple_of(j * 2 * DH, 128), 2 * DH), :], wo_v.at[slot], s_wo.at[slot]),
        )

    cp_x = pltpu.make_async_copy(x_hbm, x_v, s_misc.at[0])
    cp_c = pltpu.make_async_copy(c_hbm, c_v, s_misc.at[1])
    cp_ma = pltpu.make_async_copy(wm_hbm.at[:, pl.ds(0, HM)], wm_v.at[0], s_misc.at[2])
    cp_mb = pltpu.make_async_copy(wm_hbm.at[:, pl.ds(HM, HM)], wm_v.at[1], s_misc.at[3])
    cp_g = pltpu.make_async_copy(wg_hbm, wg_v, s_misc.at[4])
    cp_u = pltpu.make_async_copy(wu_hbm, wu_v, s_misc.at[5])
    cp_d = pltpu.make_async_copy(wd_hbm, wd_v, s_misc.at[6])

    cp_c.start()
    cp_x.start()
    cp_ma.start()
    for j in range(NB):
        for cp in pair_copies(j, j):
            cp.start()

    cp_c.wait()
    cp_x.wait()
    cp_ma.wait()
    x = x_v[0].astype(f32)
    c = c_v[...].astype(f32)
    sc = _rows(_r(jax.nn.silu(c))).astype(bf16)
    if mode != "dma":
        mod_a = _r(_dot(sc, wm_v[0]))
    else:
        mod_a = jnp.zeros((8, HM), f32)
    sa, ca, ga = mod_a[:, :D], mod_a[:, D:2 * D], mod_a[:, 2 * D:]
    x8 = _rows(x)
    h = _r(_r(_r(_ln(x8)) * _r(1.0 + ca)) + sa).astype(bf16)
    scale = DH ** -0.5

    def body(j, acc):
        slot = lax.rem(j, NB)
        cq, ck, cv, co = pair_copies(j, slot)
        cq.wait()
        ck.wait()
        cv.wait()
        co.wait()
        if mode != "dma":
            q2 = _dot(h, wq_v[slot]).astype(bf16)
            outs = []
            for t in range(2):
                q = q2[:, t * DH:(t + 1) * DH]
                s = _dot(q, k_v[slot, t]) * scale
                m = jnp.max(s, axis=-1, keepdims=True)
                e = jnp.exp(s - m)
                l = jnp.sum(e, axis=-1, keepdims=True)
                p = (e / l).astype(bf16)
                o = lax.dot_general(p, v_v[slot, t], (((1,), (1,)), ((), ())),
                                    preferred_element_type=f32)
                outs.append(o)
            o2 = jnp.concatenate(outs, axis=-1).astype(bf16)
            acc = acc + _dot(o2, wo_v[slot])

        @pl.when(j + NB < NP)
        def _():
            for cp in pair_copies(j + NB, slot):
                cp.start()

        @pl.when(j + NB == NP)
        def _():
            cp_mb.start()
            cp_g.start()
            cp_u.start()
            cp_d.start()
        return acc

    acc = lax.fori_loop(0, NP, body, jnp.zeros((8, D), f32))
    x1 = _r(x8 + _r(ga * _r(acc)))
    cp_mb.wait()
    cp_g.wait()
    cp_u.wait()
    cp_d.wait()
    if mode != "dma":
        mod_b = _r(_dot(sc, wm_v[1]))
        sb, cb, gb = mod_b[:, :D], mod_b[:, D:2 * D], mod_b[:, 2 * D:]
        h2 = _r(_r(_r(_ln(x1)) * _r(1.0 + cb)) + sb).astype(bf16)
        g = _r(_dot(h2, wg_v[...]))
        u = _r(_dot(h2, wu_v[...]))
        a = _r(_r(jax.nn.gelu(g, approximate=True)) * u).astype(bf16)
        y = x1 + _r(gb * _r(_dot(a, wd_v[...])))
    else:
        y = x1
    o_ref[0] = y[0:1].astype(bf16)


def _call(mode, A_x, A_k_cache, A_v_cache, A_wq, A_wo, B_w_gate, B_w_up, B_w_down, c, w_mod):
    kT = jnp.swapaxes(A_k_cache[0], 1, 2)
    vT = jnp.swapaxes(A_v_cache[0], 1, 2)
    any_spec = pl.BlockSpec(memory_space=pl.ANY)
    return pl.pallas_call(
        functools.partial(_kernel, mode),
        out_shape=jax.ShapeDtypeStruct((1, 1, D), bf16),
        in_specs=[any_spec] * 10,
        out_specs=pl.BlockSpec(memory_space=pltpu.VMEM),
        scratch_shapes=[
            pltpu.VMEM((1, 1, D), bf16),
            pltpu.VMEM((1, D), bf16),
            pltpu.VMEM((2, D, 3 * D), bf16),
            pltpu.VMEM((NB, D, 2 * DH), bf16),
            pltpu.VMEM((NB, 2, DH, W), bf16),
            pltpu.VMEM((NB, 2, DH, W), bf16),
            pltpu.VMEM((NB, 2 * DH, D), bf16),
            pltpu.VMEM((D, F), bf16),
            pltpu.VMEM((D, F), bf16),
            pltpu.VMEM((F, D), bf16),
            pltpu.SemaphoreType.DMA((7,)),
            pltpu.SemaphoreType.DMA((NB,)),
            pltpu.SemaphoreType.DMA((NB,)),
            pltpu.SemaphoreType.DMA((NB,)),
            pltpu.SemaphoreType.DMA((NB,)),
        ],
        compiler_params=pltpu.CompilerParams(vmem_limit_bytes=100 * 1024 * 1024),
    )(A_x, c, kT, vT, A_wq, A_wo, w_mod, B_w_gate, B_w_up, B_w_down)


@jax.jit
def pallas_adaLN_cond__sliding_block_cached__geglu_ffn__decode_kernel(
    A_x: jax.Array,
    A_k_cache: jax.Array,
    A_v_cache: jax.Array,
    A_wq: jax.Array,
    A_wo: jax.Array,
    B_x: jax.Array,
    B_w_gate: jax.Array,
    B_w_up: jax.Array,
    B_w_down: jax.Array,
    c: jax.Array,
    w_mod: jax.Array,
):
    return _call("full", A_x, A_k_cache, A_v_cache, A_wq, A_wo, B_w_gate, B_w_up, B_w_down, c, w_mod)
```

```python
import jax
import jax.numpy as jnp
from jax import lax
import jax.experimental.pallas as pl
import jax.experimental.pallas.tpu as pltpu

D = 640
H = 32
DH = 192
SK = 32768
W = min(4096, max(256, SK // 4))
F = 1536
EPS = 1e-5
HC = 2
NB = 2
DOFF = (0, 640, 1024, 1280, 1408, F)
ND = len(DOFF) - 1
f32 = jnp.float32
bf16 = jnp.bfloat16


def _ln(x):
    m = jnp.mean(x, axis=-1, keepdims=True)
    d = x - m
    v = jnp.mean(d * d, axis=-1, keepdims=True)
    return d / jnp.sqrt(v + EPS)


def _rows(x):
    return jnp.broadcast_to(x, (8, x.shape[-1]))


def _dot(a, b):
    return jnp.dot(a, b, preferred_element_type=f32)


def _r(x):
    return x.astype(bf16).astype(f32)


def _kernel(x_hbm, c_hbm, k_hbm, v_hbm, wq_hbm, wo_hbm, wm_hbm, wg_hbm, wu_hbm, wd_hbm,
            o_ref,
            x_v, c_v, wm_v, wq_v, k_v, v_v, wo_v, wg_v, wu_v, wd_v, q_s, o_s,
            s_misc, s_k, s_v):
    NG = H // HC
    GW = HC * DH

    def k_copy(j, slot):
        return pltpu.make_async_copy(k_hbm.at[pl.ds(j * HC, HC), :, pl.ds(SK - W, W)], k_v.at[slot], s_k.at[slot])

    def v_copy(j, slot):
        return pltpu.make_async_copy(v_hbm.at[pl.ds(j * HC, HC), :, pl.ds(SK - W, W)], v_v.at[slot], s_v.at[slot])

    cp_x = pltpu.make_async_copy(x_hbm, x_v, s_misc.at[0])
    cp_c = pltpu.make_async_copy(c_hbm, c_v, s_misc.at[1])
    cp_m = pltpu.make_async_copy(wm_hbm, wm_v, s_misc.at[2])
    cp_q = pltpu.make_async_copy(wq_hbm, wq_v, s_misc.at[3])
    cp_o = pltpu.make_async_copy(wo_hbm, wo_v, s_misc.at[4])
    cp_g = pltpu.make_async_copy(wg_hbm, wg_v, s_misc.at[5])
    cp_u = pltpu.make_async_copy(wu_hbm, wu_v, s_misc.at[6])
    cp_d = [pltpu.make_async_copy(wd_hbm.at[pl.ds(DOFF[i], DOFF[i + 1] - DOFF[i])], wd_v.at[pl.ds(DOFF[i], DOFF[i + 1] - DOFF[i])], s_misc.at[7 + i])
            for i in range(ND)]

    cp_c.start()
    cp_x.start()
    cp_m.start()
    cp_q.start()
    for j in range(NB):
        k_copy(j, j).start()
        v_copy(j, j).start()

    cp_c.wait()
    cp_x.wait()
    x8 = _rows(x_v[0].astype(f32))
    sc = _rows(_r(jax.nn.silu(c_v[...].astype(f32)))).astype(bf16)
    ln_x = _r(_ln(x8))
    cp_m.wait()
    mod = _r(_dot(sc, wm_v[...]))
    sa, ca, ga, sb, cb, gb = (mod[:, i * D:(i + 1) * D] for i in range(6))
    h = _r(_r(ln_x * _r(1.0 + ca)) + sa).astype(bf16)
    cp_q.wait()
    for j in range(NG):
        q_s[j] = _dot(h, wq_v[:, j * GW:(j + 1) * GW]).astype(bf16)
    scale = DH ** -0.5

    def body(j, carry):
        slot = lax.rem(j, NB)
        k_copy(j, slot).wait()
        q2 = q_s[j]
        ps = []
        for t in range(HC):
            q = q2[:, t * DH:(t + 1) * DH]
            s = _dot(q, k_v[slot, t]) * scale
            m = jnp.max(s, axis=-1, keepdims=True)
            e = jnp.exp(s - m)
            l = jnp.sum(e, axis=-1, keepdims=True)
            ps.append((e / l).astype(bf16))

        @pl.when(j + NB < NG)
        def _():
            k_copy(j + NB, slot).start()

        v_copy(j, slot).wait()
        outs = [lax.dot_general(ps[t], v_v[slot, t], (((1,), (1,)), ((), ())),
                                preferred_element_type=f32) for t in range(HC)]
        o_s[j] = jnp.concatenate(outs, axis=-1).astype(bf16)

        @pl.when(j + NB < NG)
        def _():
            v_copy(j + NB, slot).start()

        @pl.when(j + NB == NG)
        def _():
            cp_o.start()
            cp_g.start()
            cp_u.start()
            for cp in cp_d:
                cp.start()
        return carry

    lax.fori_loop(0, NG, body, 0)

    cp_o.wait()
    acc = jnp.zeros((8, D), f32)
    for j in range(NG):
        acc = acc + _dot(o_s[j], wo_v[j * GW:(j + 1) * GW, :])
    x1 = _r(x8 + _r(ga * _r(acc)))
    h2 = _r(_r(_r(_ln(x1)) * _r(1.0 + cb)) + sb).astype(bf16)
    cp_g.wait()
    g = _r(_dot(h2, wg_v[...]))
    cp_u.wait()
    u = _r(_dot(h2, wu_v[...]))
    a = _r(_r(jax.nn.gelu(g, approximate=True)) * u).astype(bf16)
    f = jnp.zeros((8, D), f32)
    a_col = jnp.broadcast_to(a[0:1, DOFF[-2]:].astype(f32), (128, F - DOFF[-2])).T
    a_col = jnp.concatenate([a_col] * (D // 128), axis=1)
    for i in range(ND - 1):
        cp_d[i].wait()
        f = f + _dot(a[:, DOFF[i]:DOFF[i + 1]], wd_v[DOFF[i]:DOFF[i + 1], :])
    cp_d[ND - 1].wait()
    f = f + jnp.sum(a_col * wd_v[DOFF[-2]:, :].astype(f32), axis=0, keepdims=True)
    y = x1 + _r(gb * _r(f))
    o_ref[0] = y[0:1].astype(bf16)


def _call(A_x, A_k_cache, A_v_cache, A_wq, A_wo, B_w_gate, B_w_up, B_w_down, c, w_mod):
    kT = jnp.swapaxes(A_k_cache[0], 1, 2)
    vT = jnp.swapaxes(A_v_cache[0], 1, 2)
    any_spec = pl.BlockSpec(memory_space=pl.ANY)
    return pl.pallas_call(
        _kernel,
        out_shape=jax.ShapeDtypeStruct((1, 1, D), bf16),
        in_specs=[any_spec] * 10,
        out_specs=pl.BlockSpec(memory_space=pltpu.VMEM),
        scratch_shapes=[
            pltpu.VMEM((1, 1, D), bf16),
            pltpu.VMEM((1, D), bf16),
            pltpu.VMEM((D, 6 * D), bf16),
            pltpu.VMEM((D, H * DH), bf16),
            pltpu.VMEM((NB, HC, DH, W), bf16),
            pltpu.VMEM((NB, HC, DH, W), bf16),
            pltpu.VMEM((H * DH, D), bf16),
            pltpu.VMEM((D, F), bf16),
            pltpu.VMEM((D, F), bf16),
            pltpu.VMEM((F, D), bf16),
            pltpu.VMEM((H // HC, 8, HC * DH), bf16),
            pltpu.VMEM((H // HC, 8, HC * DH), bf16),
            pltpu.SemaphoreType.DMA((7 + ND,)),
            pltpu.SemaphoreType.DMA((NB,)),
            pltpu.SemaphoreType.DMA((NB,)),
        ],
        compiler_params=pltpu.CompilerParams(vmem_limit_bytes=100 * 1024 * 1024),
    )(A_x, c, kT, vT, A_wq, A_wo, w_mod, B_w_gate, B_w_up, B_w_down)


@jax.jit
def pallas_adaLN_cond__sliding_block_cached__geglu_ffn__decode_kernel(
    A_x: jax.Array,
    A_k_cache: jax.Array,
    A_v_cache: jax.Array,
    A_wq: jax.Array,
    A_wo: jax.Array,
    B_x: jax.Array,
    B_w_gate: jax.Array,
    B_w_up: jax.Array,
    B_w_down: jax.Array,
    c: jax.Array,
    w_mod: jax.Array,
):
    return _call(A_x, A_k_cache, A_v_cache, A_wq, A_wo, B_w_gate, B_w_up, B_w_down, c, w_mod)
```
